```python
import jax
import jax.numpy as jnp

def _softmax(x, axis=-1):
    return jax.nn.softmax(x, axis=axis)
def _gelu(x):
    return jax.nn.gelu(x, approximate=True)
def _silu(x):
    return jax.nn.silu(x)
def _sigmoid(x):
    return jax.nn.sigmoid(x)
def _layernorm(x, axis=-1, eps=1e-5):
    m = jnp.mean(x, axis=axis, keepdims=True)
    v = jnp.var(x, axis=axis, keepdims=True)
    return (x - m) / jnp.sqrt(v + eps)
def _scatter_add(tgt, idx, src, axis=0):
    return tgt.at[idx].add(src)
def _segment_sum(src, seg, n):
    return jax.ops.segment_sum(src, seg, n)
class _Rng:
    def __init__(self, key):
        self._k = key
    def _next(self):
        self._k, sub = jax.random.split(self._k)
        return sub
    def normal(self, shape):
        return jax.random.normal(self._next(), shape, dtype=jnp.bfloat16)
    def randint(self, lo, hi, shape):
        return jax.random.randint(self._next(), shape, lo, hi, dtype=jnp.int32)
    def uniform(self, shape, lo=0.0, hi=1.0):
        return jax.random.uniform(self._next(), shape, jnp.bfloat16, lo, hi)
    def permutation(self, n):
        return jax.random.permutation(self._next(), n)


kernel_name = 'concat_heads__gqa_block_cached__mha_block_cached__near_ridge'

def setup_inputs():
    _rng = _Rng(jax.random.key(int.from_bytes(__import__("os").urandom(4), "little")))
    _w = (lambda a: (lambda t: t.astype(jnp.bfloat16) if jnp.issubdtype(t.dtype, jnp.floating) else t)(jnp.asarray(a)))
    def _A_setup():
        B, Sq, D = 16, 160, 640
        Hq, Hkv, Sk, Dh = 32, 32, 512, 192
        assert Hq % Hkv == 0, (Hq, Hkv)
        return {
            "x": _w((lambda *s: _rng.normal(s) * 0.05)(B, Sq, D)),
            "k_cache": _w((lambda *s: _rng.normal(s) * 0.05)(B, Hkv, Sk, Dh)),
            "v_cache": _w((lambda *s: _rng.normal(s) * 0.05)(B, Hkv, Sk, Dh)),
            "wq": _w((lambda *s: _rng.normal(s) * 0.05)(D, Hq * Dh) * (D ** -0.5)),
            "wo": _w((lambda *s: _rng.normal(s) * 0.05)(Hq * Dh, D) * ((Hq * Dh) ** -0.5)),
        }
    _A_in = _A_setup()

    def _B_setup():
        B, Sq, D = 16, 160, 640
        H, Sk, Dh = 32, 512, 192
        return {
            "x": _w((lambda *s: _rng.normal(s) * 0.05)(B, Sq, D)),
            "k_cache": _w((lambda *s: _rng.normal(s) * 0.05)(B, H, Sk, Dh)),
            "v_cache": _w((lambda *s: _rng.normal(s) * 0.05)(B, H, Sk, Dh)),
            "wq": _w((lambda *s: _rng.normal(s) * 0.05)(D, H * Dh) * (D ** -0.5)),
            "wo": _w((lambda *s: _rng.normal(s) * 0.05)(H * Dh, D) * ((H * Dh) ** -0.5)),
        }
    _B_in = _B_setup()

    return {
        "A_x": _A_in["x"],
        "A_k_cache": _A_in["k_cache"],
        "A_v_cache": _A_in["v_cache"],
        "A_wq": _A_in["wq"],
        "A_wo": _A_in["wo"],
        "B_x": _B_in["x"],
        "B_k_cache": _B_in["k_cache"],
        "B_v_cache": _B_in["v_cache"],
        "B_wq": _B_in["wq"],
        "B_wo": _B_in["wo"],
    }

def reference(A_x, A_k_cache, A_v_cache, A_wq, A_wo, B_x, B_k_cache, B_v_cache, B_wq, B_wo):
    def _A_ref(x, k_cache, v_cache, wq, wo):
        B, Sq, D = x.shape
        Hq, Dh = 32, 192
        Hkv = k_cache.shape[1]
        rep = Hq // Hkv
        q = (lambda x, *d: x.transpose(*d))((x @ wq).reshape(B, Sq, Hq, Dh), 0, 2, 1, 3)
        k = jnp.repeat(k_cache, rep, axis=1)
        v = jnp.repeat(v_cache, rep, axis=1)
        scores = jnp.einsum("bhqd,bhkd->bhqk", q, k) * (Dh ** -0.5)
        p = _softmax(scores, axis=-1)
        o = jnp.einsum("bhqk,bhkd->bhqd", p, v)
        return (lambda x, *d: x.transpose(*d))(o, 0, 2, 1, 3).reshape(B, Sq, Hq * Dh) @ wo

    def _B_ref(x, k_cache, v_cache, wq, wo):
        B, Sq, D = x.shape
        H, Dh = 32, 192
        q = (lambda x, *d: x.transpose(*d))((x @ wq).reshape(B, Sq, H, Dh), 0, 2, 1, 3)
        scores = jnp.einsum("bhqd,bhkd->bhqk", q, k_cache) * (Dh ** -0.5)
        p = _softmax(scores, axis=-1)
        o = jnp.einsum("bhqk,bhkd->bhqd", p, v_cache)
        return (lambda x, *d: x.transpose(*d))(o, 0, 2, 1, 3).reshape(B, Sq, H * Dh) @ wo

    a = _A_ref(A_x, A_k_cache, A_v_cache, A_wq, A_wo)
    b = _B_ref(B_x, B_k_cache, B_v_cache, B_wq, B_wo)
    return jnp.concatenate([a, b], axis=-1)
```

```python
import functools
import jax
import jax.numpy as jnp
import jax.experimental.pallas as pl
import jax.experimental.pallas.tpu as pltpu

NT = (((1,), (1,)), ((), ()))


def make(hg=2, vmem_mb=100, look=1, hybrid=0, flags=None, prenorm=0):
    B, Sq, D, H, Sk, Dh = 16, 160, 640, 32, 512, 192
    G = H // hg
    scale = Dh ** -0.5
    f32, bf16 = jnp.float32, jnp.bfloat16

    def kernel(ax, ak, av, awq, awo, bx, bk, bv, bwq, bwo, out_ref, acc_ref):
        g = pl.program_id(0)
        b = pl.program_id(1)
        xs, ks, vs, wqs, wos = (ax, bx), (ak, bk), (av, bv), (awq, bwq), (awo, bwo)

        @pl.when(g == 0)
        def _():
            acc_ref[b] = jnp.zeros((Sq, 2 * D), f32)

        qs = []
        for br in range(2):
            q = jnp.dot(xs[br][b], wqs[br][...], preferred_element_type=f32)
            qs.append((q * scale).astype(bf16))

        items = [(br, h) for br in range(2) for h in range(hg)]
        n = len(items)
        S = {}
        O = {}

        def qk(i):
            br, h = items[i]
            S[i] = jnp.dot(qs[br][:, h * Dh:(h + 1) * Dh], ks[br][0, h], preferred_element_type=f32)

        def pv(i):
            br, h = items[i]
            s = S.pop(i)
            m = jnp.max(s, axis=-1, keepdims=True)
            p = jnp.exp(s - m)
            l = jnp.sum(p, axis=-1, keepdims=True)
            r = 1.0 / l
            vt = vs[br][0, h]
            if hybrid:
                if prenorm:
                    p = p * r
                p = p.astype(bf16)
                ot = jax.lax.dot_general(vt, p[:128], NT, preferred_element_type=f32)
                orem = jax.lax.dot_general(p[128:], vt, NT, preferred_element_type=f32)
                if prenorm:
                    O[i] = (ot.astype(bf16), orem.astype(bf16))
                else:
                    o = jnp.concatenate([ot.T, orem], axis=0)
                    O[i] = (o * r).astype(bf16)
            else:
                o = jax.lax.dot_general(p.astype(bf16), vt, NT, preferred_element_type=f32)
                O[i] = (o * r).astype(bf16)

        def oproj(br):
            os_ = [O.pop(br * hg + h) for h in range(hg)]
            if hybrid and prenorm:
                ot = jnp.concatenate([a for a, _ in os_], axis=0)
                orem = jnp.concatenate([c for _, c in os_], axis=1)
                o = jnp.concatenate([ot.T, orem], axis=0)
            else:
                o = jnp.concatenate(os_, axis=-1)
            y = jnp.dot(o, wos[br][...], preferred_element_type=f32)
            acc_ref[b, :, br * D:(br + 1) * D] += y

        for i in range(min(look, n)):
            qk(i)
        for i in range(n):
            if i + look < n:
                qk(i + look)
            if i == n - 1:
                oproj(0)
            pv(i)
        oproj(1)

        @pl.when(g == G - 1)
        def _():
            out_ref[0] = acc_ref[b].astype(out_ref.dtype)

    x_spec = pl.BlockSpec((B, Sq, D), lambda g, b: (0, 0, 0))
    kv_spec = pl.BlockSpec((1, hg, Dh, Sk), lambda g, b: (b, g, 0, 0))
    wq_spec = pl.BlockSpec((D, hg * Dh), lambda g, b: (0, g))
    wo_spec = pl.BlockSpec((hg * Dh, D), lambda g, b: (g, 0))
    out_spec = pl.BlockSpec((1, Sq, 2 * D), lambda g, b: (jnp.where(g == G - 1, b, 0), 0, 0))

    def fn(A_x, A_k, A_v, A_wq, A_wo, B_x, B_k, B_v, B_wq, B_wo):
        t = lambda a: jnp.swapaxes(a, 2, 3)
        return pl.pallas_call(
            kernel,
            grid=(G, B),
            in_specs=[x_spec, kv_spec, kv_spec, wq_spec, wo_spec] * 2,
            out_specs=out_spec,
            out_shape=jax.ShapeDtypeStruct((B, Sq, 2 * D), jnp.bfloat16),
            scratch_shapes=[pltpu.VMEM((B, Sq, 2 * D), jnp.float32)],
            compiler_params=pltpu.CompilerParams(
                dimension_semantics=("arbitrary", "arbitrary"),
                vmem_limit_bytes=vmem_mb * 1024 * 1024, flags=flags),
        )(A_x, t(A_k), t(A_v), A_wq, A_wo, B_x, t(B_k), t(B_v), B_wq, B_wo)
    return fn


@jax.jit
def pallas_concat_heads__gqa_block_cached__mha_block_cached__near_ridge_kernel(
    A_x, A_k_cache, A_v_cache, A_wq, A_wo, B_x, B_k_cache, B_v_cache, B_wq, B_wo
):
    return make(hg=8, hybrid=1, look=2)(
        A_x, A_k_cache, A_v_cache, A_wq, A_wo, B_x, B_k_cache, B_v_cache, B_wq, B_wo)
```

```python
import contextlib
import functools
import math
import jax
import jax.numpy as jnp
from jax import lax
import jax.experimental.pallas as pl
import jax.experimental.pallas.tpu as pltpu

NT = (((1,), (1,)), ((), ()))


def make(vmem_mb=120, look=2, flags=None, olag=2, masktrick=0, nslot=3, rc=16, qpos=0, qlast=1, order=0,
         tlook=2, tolag=2, NQ=5, TS=2, NB0=2, prof=0, L=4, sumb=1, pbuf=1, qla=1, only=0, spos=-1):
    B, Sq, D, H, Sk, Dh = 16, 160, 640, 32, 512, 192
    P = H // 2
    W = 2 * Dh
    NB = B // L
    NBT = NB // TS
    T = 2 * P - L
    NW = 8
    NS = 4
    C0 = B // NB0
    qscale = (Dh ** -0.5) * math.log2(math.e)
    f32, bf16 = jnp.float32, jnp.bfloat16
    SM = 128
    scope = (lambda n: jax.named_scope(n)) if prof else (lambda n: contextlib.nullcontext())

    def kernel(ax, ak, av, awq, awo, bx, bk, bv, bwq, bwo, out,
               xb, kb, vb, wqb, wob, qb, acc, ob, p_s, sem_k, sem_v, sem_x, sem_wq, sem_wo, sem_o):
        xs, ks, vs, wqs, wos = (ax, bx), (ak, bk), (av, bv), (awq, bwq), (awo, bwo)

        def kv_main(br, p, slot):
            return (pltpu.make_async_copy(ks[br].at[:, p], kb.at[slot], sem_k.at[slot]),
                    pltpu.make_async_copy(vs[br].at[:, p], vb.at[slot], sem_v.at[slot]))

        def kv_tail(c, slot):
            cps = []
            for i in range(NB):
                cps.append(pltpu.make_async_copy(bk.at[c * NB + i, pl.ds(P - L, L)], kb.at[slot, pl.ds(i * L, L)], sem_k.at[slot]))
                cps.append(pltpu.make_async_copy(bv.at[c * NB + i, pl.ds(P - L, L)], vb.at[slot, pl.ds(i * L, L)], sem_v.at[slot]))
            return cps

        def kv_wait(slot):
            pltpu.make_async_copy(kb.at[slot], kb.at[slot], sem_k.at[slot]).wait()
            pltpu.make_async_copy(vb.at[slot], vb.at[slot], sem_v.at[slot]).wait()

        def xa_copy(c):
            return pltpu.make_async_copy(ax.at[pl.ds(c * NB0, NB0)], xb.at[0, pl.ds(c * NB0, NB0)], sem_x.at[c])

        def xb_copy():
            return pltpu.make_async_copy(bx, xb.at[1], sem_x.at[C0])

        def wq_copy(br, p, wslot):
            col = p * W if isinstance(p, int) else pl.multiple_of(p * W, 128)
            return pltpu.make_async_copy(wqs[br].at[:, pl.ds(col, W)], wqb.at[wslot], sem_wq.at[wslot])

        def wo_copy(br, p, wslot):
            return pltpu.make_async_copy(wos[br].at[p], wob.at[wslot], sem_wo.at[wslot])

        def o_copy(b):
            return pltpu.make_async_copy(ob.at[b], out.at[b], sem_o.at[b])

        lane = lax.broadcasted_iota(jnp.int32, (Sq, 128), 1)

        def qproj(x, w):
            q = jnp.dot(x, w, preferred_element_type=f32)
            return (q * qscale).astype(bf16)

        def attention_block(U, load_k, load_v, load_q, load_wo, finish, filler, look, olag):
            Q, S, R, OT, OR, ON, PP = {}, {}, {}, {}, {}, {}, {}

            def qk(n):
                u, h = divmod(n, 2)
                q = Q[u]
                if h == 0:
                    S[n] = jnp.dot(q[:, :Dh], load_k(u, 0, Dh), preferred_element_type=f32)
                elif masktrick:
                    t1 = jnp.where(lane >= 64, q[:, 128:256], jnp.zeros((), bf16))
                    S[n] = jnp.dot(jnp.concatenate([t1, q[:, 256:]], axis=1), load_k(u, 128, W),
                                   preferred_element_type=f32)
                else:
                    S[n] = jnp.dot(q[:, Dh:], load_k(u, Dh, W), preferred_element_type=f32)

            def softmax(n):
                rs, ps = [], []
                sn = S.pop(n)
                for r0 in range(0, Sq, rc):
                    s = sn[r0:r0 + rc]
                    m = jnp.max(s, axis=-1, keepdims=True)
                    e = jnp.exp2(s - m)
                    p = e.astype(bf16)
                    l = jnp.sum(p.astype(f32) if sumb else e, axis=-1, keepdims=True)
                    rs.append(1.0 / l)
                    if pbuf:
                        p_s[n % NS, r0:r0 + rc, :] = p
                    else:
                        ps.append(p)
                R[n] = jnp.concatenate(rs, axis=0)
                if not pbuf:
                    PP[n] = jnp.concatenate(ps, axis=0)

            def pv(n):
                u, h = divmod(n, 2)
                if pbuf:
                    pm, pr = p_s[n % NS, :SM, :], p_s[n % NS, SM:, :]
                else:
                    p = PP.pop(n)
                    pm, pr = p[:SM], p[SM:]
                vt = load_v(u, h * Dh, (h + 1) * Dh)
                if order == 0:
                    OT[n] = lax.dot_general(vt, pm, NT, preferred_element_type=f32)
                    OR[n] = lax.dot_general(pr, vt, NT, preferred_element_type=f32)
                else:
                    OR[n] = lax.dot_general(pr, vt, NT, preferred_element_type=f32)
                    OT[n] = lax.dot_general(vt, pm, NT, preferred_element_type=f32)

            def onorm(u):
                ot = jnp.concatenate([OT.pop(2 * u), OT.pop(2 * u + 1)], axis=0)
                orem = jnp.concatenate([OR.pop(2 * u), OR.pop(2 * u + 1)], axis=1)
                o = jnp.concatenate([ot.T, orem], axis=0)
                r0, r1 = R.pop(2 * u), R.pop(2 * u + 1)
                o = jnp.concatenate([o[:, :128] * r0, o[:, 128:256] * jnp.where(lane < 64, r0, r1), o[:, 256:] * r1], axis=1)
                ON[u] = o.astype(bf16)

            def oproj(u):
                finish(u, jnp.dot(ON.pop(u), load_wo(u), preferred_element_type=f32))

            N = 2 * U
            nload = 0

            def need_q(u):
                nonlocal nload
                while nload <= min(u, U - 1):
                    Q[nload] = load_q(nload)
                    nload += 1

            need_q((look - 1) // 2)
            nf = 0
            for n in range(look):
                qk(n)
            no = 0
            for n in range(N):
                if n % 2 == qpos and filler and nf < U - qlast:
                    need_q((n + look + 1) // 2 + qla)
                    filler(nf)
                    nf += 1
                if n + look < N:
                    need_q((n + look) // 2)
                    qk(n + look)
                if n % 2 == 0 and n >= 2:
                    onorm(n // 2 - 1)
                if n % 2 == 1 and n // 2 - olag >= no:
                    oproj(no)
                    no += 1
                softmax(n)
                pv(n)
            while no < U - 1:
                oproj(no)
                no += 1
            onorm(U - 1)
            oproj(U - 1)
            while filler and nf < U:
                filler(nf)
                nf += 1

        xa_copy(0).start()
        for j in range(L):
            wq_copy(0, j, j).start()
        with scope("w_first"):
            for j in range(L):
                wq_copy(0, j, j).wait()
        for c in range(1, C0):
            xa_copy(c).start()

        def start_chunk(t, slot):
            for cp in kv_main(0, t, slot):
                cp.start()
            wo_copy(0, t, t % NW).start()
            wq_copy(0, t + L, (t + L) % NW).start()

        def phase0(c, carry):
            with scope("w_x"):
                xa_copy(c).wait()

            @pl.when(c == 1)
            def _():
                start_chunk(0, 0)

            for i in range(NB0):
                b = c * NB0 + i
                for j in range(L):
                    qb[j, b] = qproj(xb[0, b], wqb[j])
                acc[0, b] = jnp.zeros((Sq, D), f32)
                acc[1, b] = jnp.zeros((Sq, D), f32)
            return carry

        lax.fori_loop(0, C0, phase0, 0)
        for t0 in range(1, nslot - 1):
            start_chunk(t0, t0)
        xb_copy().start()

        def main(t, carry):
            slot, qr, qw = carry
            tn = t + (nslot - 1)
            nslot_i = jnp.where(slot == 0, nslot - 1, slot - 1)

            def starts():
                for br in range(2):
                    @pl.when(jnp.logical_and(tn >= br * P, tn < min((br + 1) * P, T)))
                    def _():
                        for cp in kv_main(br, tn - br * P, nslot_i):
                            cp.start()
                        wo_copy(br, tn - br * P, tn & (NW - 1)).start()

                    @pl.when(jnp.logical_and(tn + L >= br * P, tn + L < (br + 1) * P))
                    def _():
                        wq_copy(br, tn + L - br * P, (tn + L) & (NW - 1)).start()

                @pl.when(tn >= T)
                def _():
                    for cp in kv_tail(tn - T, nslot_i):
                        cp.start()

                @pl.when(tn == T)
                def _():
                    for j in range(L):
                        wo_copy(1, P - L + j, (T + j) % NW).start()

            if spos < 0:
                starts()

            @pl.when(t == P - L)
            def _():
                xb_copy().wait()

            with scope("w_main"):
                wo_copy(0, 0, t & (NW - 1)).wait()
                wq_copy(0, 0, (t + L) & (NW - 1)).wait()
                kv_wait(slot)

            br = t >> 4
            brq = (t + L) >> 4

            def finish(u, y):
                acc[br, u] += y

            def filler(u):
                if u == spos:
                    starts()
                qb[qw, u] = qproj(xb[brq, u], wqb[(t + L) & (NW - 1)])

            attention_block(B, lambda u, a, b: kb[slot, u, a:b, :], lambda u, a, b: vb[slot, u, a:b, :],
                            lambda u: qb[qr, u], lambda u: wob[t & (NW - 1)], finish, filler, look, olag)
            inc = lambda v, n: jnp.where(v == n - 1, 0, v + 1)
            return inc(slot, nslot), inc(qr, NQ), inc(qw, NQ)

        if only != 2:
          lax.fori_loop(0, T, main, (jnp.int32(0), jnp.int32(0), jnp.int32(L % NQ)))

        for j in range(L):
            wo_copy(1, P - L + j, (T + j) % NW).wait()

        def tail(it, slot):
            c = it // TS
            sub = it - c * TS
            cn = c + (nslot - 1)

            @pl.when(sub == 0)
            def _():
                @pl.when(cn < L)
                def _():
                    for cp in kv_tail(cn, jnp.where(slot == 0, nslot - 1, slot - 1)):
                        cp.start()
                with scope("w_tail"):
                    kv_wait(slot)

            u0 = sub * (NBT * L)

            def finish(u, y):
                i, j = divmod(u, L)
                b = it * NBT + i
                if j < L - 1:
                    acc[1, b] += y
                else:
                    ob[b, :, :D] = acc[0, b].astype(bf16)
                    ob[b, :, D:] = (acc[1, b] + y).astype(bf16)
                    o_copy(b).start()

            attention_block(NBT * L, lambda u, a, b: kb[slot, u0 + u, a:b, :], lambda u, a, b: vb[slot, u0 + u, a:b, :],
                            lambda u: qb[(T + u % L) % NQ, it * NBT + u // L],
                            lambda u: wob[(T + u % L) % NW], finish, None, tlook, tolag)
            nxt = jnp.where(slot == nslot - 1, 0, slot + 1)
            return jnp.where(sub == TS - 1, nxt, slot)

        if only != 1:
            lax.fori_loop(0, L * TS, tail, jnp.int32(T % nslot))
        with scope("w_out"):
            for b in range(B):
                o_copy(b).wait()

    hbm = pl.BlockSpec(memory_space=pl.ANY)

    def fn(A_x, A_k, A_v, A_wq, A_wo, B_x, B_k, B_v, B_wq, B_wo):
        t = lambda a: jnp.swapaxes(a, 2, 3).reshape(B, P, W, Sk)
        w = lambda a: a.reshape(P, W, D)
        DMA = pltpu.SemaphoreType.DMA
        return pl.pallas_call(
            kernel,
            in_specs=[hbm] * 10,
            out_specs=hbm,
            out_shape=jax.ShapeDtypeStruct((B, Sq, 2 * D), bf16),
            scratch_shapes=[
                pltpu.VMEM((2, B, Sq, D), bf16),
                pltpu.VMEM((nslot, B, W, Sk), bf16),
                pltpu.VMEM((nslot, B, W, Sk), bf16),
                pltpu.VMEM((NW, D, W), bf16),
                pltpu.VMEM((NW, W, D), bf16),
                pltpu.VMEM((NQ, B, Sq, W), bf16),
                pltpu.VMEM((2, B, Sq, D), f32),
                pltpu.VMEM((B, Sq, 2 * D), bf16),
                pltpu.VMEM((NS, Sq, Sk), bf16),
                DMA((nslot,)), DMA((nslot,)), DMA((C0 + 1,)), DMA((NW,)), DMA((NW,)), DMA((B,)),
            ],
            compiler_params=pltpu.CompilerParams(
                vmem_limit_bytes=vmem_mb * 1024 * 1024, flags=flags, disable_bounds_checks=True),
        )(A_x, t(A_k), t(A_v), A_wq, w(A_wo), B_x, t(B_k), t(B_v), B_wq, w(B_wo))
    return fn


@jax.jit
def pallas_concat_heads__gqa_block_cached__mha_block_cached__near_ridge_kernel(
    A_x, A_k_cache, A_v_cache, A_wq, A_wo, B_x, B_k_cache, B_v_cache, B_wq, B_wo
):
    return make(qla=0,qlast=2,spos=1)(
        A_x, A_k_cache, A_v_cache, A_wq, A_wo, B_x, B_k_cache, B_v_cache, B_wq, B_wo)
```

```python
import contextlib
import functools
import math
import jax
import jax.numpy as jnp
from jax import lax
import jax.experimental.pallas as pl
import jax.experimental.pallas.tpu as pltpu

NT = (((1,), (1,)), ((), ()))


def schedule(U, pattern, look, olag, qlast, has_filler):
    N = 2 * U
    ops = [("K", n) for n in range(look)]
    nk, nv, no, nf = look, 0, 0, 0
    i = 0
    while nv < N:
        c = pattern[i % len(pattern)]
        i += 1
        if c == "K" and nk < N:
            ops.append(("K", nk)); nk += 1
        elif c == "V":
            ops.append(("V", nv)); nv += 1
        elif c == "O" and 2 * (no + 1) + olag <= nv:
            ops.append(("O", no)); no += 1
        elif c == "F" and has_filler and nf < U - qlast:
            ops.append(("F", nf)); nf += 1
    ops += [("O", u) for u in range(no, U)]
    if has_filler:
        ops += [("F", u) for u in range(nf, U)]
    return ops


def make(vmem_mb=120, look=2, flags=None, olag=3, nslot=3, rc=16, qlast=2, order=0, pat="FKVKOV",
         tlook=2, tolag=3, tpat="KVKOV", NQ=5, TS=2, NB0=2, prof=0, L=4, only=0, spos=1, NS=4, qla=0, zpos=8, zboth=1, rb=0, nr=0, zk=0):
    B, Sq, D, H, Sk, Dh = 16, 160, 640, 32, 512, 192
    P = H // 2
    W = 2 * Dh
    NB = B // L
    NBT = NB // TS
    T = 2 * P - L
    NW = 8
    C0 = B // NB0
    qscale = (Dh ** -0.5) * math.log2(math.e)
    f32, bf16 = jnp.float32, jnp.bfloat16
    SM = 128
    scope = (lambda n: jax.named_scope(n)) if prof else (lambda n: contextlib.nullcontext())

    def kernel(ax, ak, av, awq, awo, bx, bk, bv, bwq, bwo, out,
               xb, kb, vb, wqb, wob, qb, acc, ob, p_s, sem_k, sem_v, sem_x, sem_wq, sem_wo, sem_o):
        xs, ks, vs, wqs, wos = (ax, bx), (ak, bk), (av, bv), (awq, bwq), (awo, bwo)

        def kv_main(br, p, slot):
            return (pltpu.make_async_copy(ks[br].at[:, p], kb.at[slot], sem_k.at[slot]),
                    pltpu.make_async_copy(vs[br].at[:, p], vb.at[slot], sem_v.at[slot]))

        def kv_tail(c, slot):
            cps = []
            for i in range(NB):
                cps.append(pltpu.make_async_copy(bk.at[c * NB + i, pl.ds(P - L, L)], kb.at[slot, pl.ds(i * L, L)], sem_k.at[slot]))
                cps.append(pltpu.make_async_copy(bv.at[c * NB + i, pl.ds(P - L, L)], vb.at[slot, pl.ds(i * L, L)], sem_v.at[slot]))
            return cps

        def kv_wait(slot):
            pltpu.make_async_copy(kb.at[slot], kb.at[slot], sem_k.at[slot]).wait()
            pltpu.make_async_copy(vb.at[slot], vb.at[slot], sem_v.at[slot]).wait()

        def xa_copy(c):
            return pltpu.make_async_copy(ax.at[pl.ds(c * NB0, NB0)], xb.at[0, pl.ds(c * NB0, NB0)], sem_x.at[c])

        def xb_copy():
            return pltpu.make_async_copy(bx, xb.at[1], sem_x.at[C0])

        def zero_copy():
            return pltpu.make_async_copy(acc.at[0], acc.at[1], sem_x.at[C0 + 1])

        def wq_copy(br, p, wslot):
            col = p * W if isinstance(p, int) else pl.multiple_of(p * W, 128)
            return pltpu.make_async_copy(wqs[br].at[:, pl.ds(col, W)], wqb.at[wslot], sem_wq.at[wslot])

        def wo_copy(br, p, wslot):
            return pltpu.make_async_copy(wos[br].at[p], wob.at[wslot], sem_wo.at[wslot])

        def o_copy(b):
            return pltpu.make_async_copy(ob.at[b], out.at[b], sem_o)

        lane = lax.broadcasted_iota(jnp.int32, (Sq, 128), 1)

        def qproj(x, w):
            q = jnp.dot(x, w, preferred_element_type=f32)
            return (q * qscale).astype(bf16)

        def attention_block(ops, load_k, load_v, load_q, load_wo, finish, filler):
            Q, S, R, OT, OR = {}, {}, {}, {}, {}

            def qk(n):
                u, h = divmod(n, 2)
                if zk and h == 1:
                    k = jnp.concatenate([jnp.zeros((64, Sk), bf16), load_k(u, h)], axis=0)
                    S[n] = jnp.dot(Q[u][:, 128:], k, preferred_element_type=f32)
                elif zk == 2:
                    k = jnp.concatenate([load_k(u, h), jnp.zeros((64, Sk), bf16)], axis=0)
                    S[n] = jnp.dot(Q[u][:, :256], k, preferred_element_type=f32)
                else:
                    S[n] = jnp.dot(Q[u][:, h * Dh:(h + 1) * Dh], load_k(u, h), preferred_element_type=f32)

            def pv(n):
                u, h = divmod(n, 2)
                rs = []
                sn = S.pop(n)
                for r0 in range(0, Sq, rc):
                    s = sn[r0:r0 + rc]
                    m = jnp.max(s, axis=-1, keepdims=True)
                    p = jnp.exp2(s - m).astype(bf16)
                    l = jnp.sum(p.astype(f32), axis=-1, keepdims=True)
                    if rb:
                        l = jnp.broadcast_to(l, (rc, 128))
                    if nr:
                        r = pl.reciprocal(l, approx=True)
                        r = r * (2.0 - l * r)
                    else:
                        r = 1.0 / l
                    rs.append(r)
                    p_s[n % NS, r0:r0 + rc, :] = p
                R[n] = jnp.concatenate(rs, axis=0)
                pm, pr = p_s[n % NS, :SM, :], p_s[n % NS, SM:, :]
                vt = load_v(u, h)
                if order == 0:
                    OT[n] = lax.dot_general(vt, pm, NT, preferred_element_type=f32)
                    OR[n] = lax.dot_general(pr, vt, NT, preferred_element_type=f32)
                elif order == 1:
                    OR[n] = lax.dot_general(pr, vt, NT, preferred_element_type=f32)
                    OT[n] = lax.dot_general(vt, pm, NT, preferred_element_type=f32)
                else:
                    ra = lax.dot_general(pr, vt[:128], NT, preferred_element_type=f32)
                    OT[n] = lax.dot_general(vt, pm, NT, preferred_element_type=f32)
                    r2 = lax.dot_general(pr, vt[128:], NT, preferred_element_type=f32)
                    OR[n] = jnp.concatenate([ra, r2], axis=1)

            def oproj(u):
                ot = jnp.concatenate([OT.pop(2 * u), OT.pop(2 * u + 1)], axis=0)
                orem = jnp.concatenate([OR.pop(2 * u), OR.pop(2 * u + 1)], axis=1)
                o = jnp.concatenate([ot.T, orem], axis=0)
                r0, r1 = R.pop(2 * u), R.pop(2 * u + 1)
                o = jnp.concatenate([o[:, :128] * r0, o[:, 128:256] * jnp.where(lane < 64, r0, r1), o[:, 256:] * r1], axis=1)
                finish(u, jnp.dot(o.astype(bf16), load_wo(u), preferred_element_type=f32))

            def need_q(n):
                if n // 2 not in Q:
                    Q[n // 2] = load_q(n // 2)

            for i, (c, n) in enumerate(ops):
                if c == "K":
                    need_q(n)
                    qk(n)
                elif c == "V":
                    pv(n)
                elif c == "O":
                    oproj(n)
                else:
                    for n2 in [m for c2, m in ops[i:] if c2 == "K"][:2 + qla]:
                        need_q(n2)
                    filler(n)

        def start_chunk(t, slot):
            for cp in kv_main(0, t, slot):
                cp.start()
            wo_copy(0, t, t % NW).start()
            wq_copy(0, t + L, (t + L) % NW).start()

        xa_copy(0).start()
        wq_copy(0, 0, 0).start()
        def zero(b, carry):
            acc[0, b] = jnp.zeros((Sq, D), f32)
            if zboth:
                acc[1, b] = jnp.zeros((Sq, D), f32)

            @pl.when(b == zpos)
            def _():
                wq_copy(0, 1, 1).start()
            return carry

        with scope("zero"):
            lax.fori_loop(0, B, zero, 0)
        with scope("w_first"):
            xa_copy(0).wait()

        def phase0a(j, carry):
            with scope("w_q"):
                wq_copy(0, j, j).wait()

            @pl.when(j + 2 < L)
            def _():
                wq_copy(0, j + 2, j + 2).start()

            @pl.when(j + 2 == L)
            def _():
                xa_copy(1).start()
                xa_copy(2).start()

            @pl.when(j + 1 == L)
            def _():
                for c in range(3, C0):
                    xa_copy(c).start()

            for b in range(NB0):
                qb[j, b] = qproj(xb[0, b], wqb[j])
            return carry

        lax.fori_loop(0, L, phase0a, 0)

        def phase0b(c, carry):
            with scope("w_x"):
                xa_copy(c).wait()

            @pl.when(c == 2)
            def _():
                start_chunk(0, 0)

            for i in range(NB0):
                b = c * NB0 + i
                for j in range(L):
                    qb[j, b] = qproj(xb[0, b], wqb[j])
            return carry

        lax.fori_loop(1, C0, phase0b, 0)
        for t0 in range(1, nslot - 1):
            start_chunk(t0, t0)
        xb_copy().start()

        def main(t, carry):
            slot, qr, qw = carry
            tn = t + (nslot - 1)
            nslot_i = jnp.where(slot == 0, nslot - 1, slot - 1)

            def starts():
                for br in range(2):
                    @pl.when(jnp.logical_and(tn >= br * P, tn < min((br + 1) * P, T)))
                    def _():
                        for cp in kv_main(br, tn - br * P, nslot_i):
                            cp.start()
                        wo_copy(br, tn - br * P, tn & (NW - 1)).start()

                    @pl.when(jnp.logical_and(tn + L >= br * P, tn + L < (br + 1) * P))
                    def _():
                        wq_copy(br, tn + L - br * P, (tn + L) & (NW - 1)).start()

                @pl.when(tn >= T)
                def _():
                    for cp in kv_tail(tn - T, nslot_i):
                        cp.start()

                @pl.when(tn == T)
                def _():
                    for j in range(L):
                        wo_copy(1, P - L + j, (T + j) % NW).start()

            @pl.when(t == P - L)
            def _():
                xb_copy().wait()

            with scope("w_main"):
                wo_copy(0, 0, t & (NW - 1)).wait()
                wq_copy(0, 0, (t + L) & (NW - 1)).wait()
                kv_wait(slot)

            br = t >> 4
            brq = (t + L) >> 4

            def finish(u, y):
                acc[br, u] += y

            def filler(u):
                if u == spos:
                    starts()
                qb[qw, u] = qproj(xb[brq, u], wqb[(t + L) & (NW - 1)])

            attention_block(schedule(B, pat, look, olag, qlast, True),
                            lambda u, h: kb[slot, u, h * Dh:(h + 1) * Dh, :],
                            lambda u, h: vb[slot, u, h * Dh:(h + 1) * Dh, :],
                            lambda u: qb[qr, u], lambda u: wob[t & (NW - 1)], finish, filler)
            inc = lambda v, n: jnp.where(v == n - 1, 0, v + 1)
            return inc(slot, nslot), inc(qr, NQ), inc(qw, NQ)

        if only != 2:
            lax.fori_loop(0, T, main, (jnp.int32(0), jnp.int32(0), jnp.int32(L % NQ)))

        for j in range(L):
            wo_copy(1, P - L + j, (T + j) % NW).wait()

        def tail(it, slot):
            c = lax.div(it, TS)
            sub = it - c * TS
            cn = c + (nslot - 1)

            @pl.when(sub == 0)
            def _():
                with scope("w_tail"):
                    kv_wait(slot)

            u0 = sub * (NBT * L)

            def finish(u, y):
                i, j = divmod(u, L)
                b = it * NBT + i
                if u == 0:
                    @pl.when(jnp.logical_and(sub == 0, cn < L))
                    def _():
                        for cp in kv_tail(cn, jnp.where(slot == 0, nslot - 1, slot - 1)):
                            cp.start()
                if j < L - 1:
                    acc[1, b] += y
                else:
                    ob[b, :, :D] = acc[0, b].astype(bf16)
                    ob[b, :, D:] = (acc[1, b] + y).astype(bf16)
                    o_copy(b).start()

            attention_block(schedule(NBT * L, tpat, tlook, tolag, 0, False),
                            lambda u, h: kb[slot, u0 + u, h * Dh:(h + 1) * Dh, :],
                            lambda u, h: vb[slot, u0 + u, h * Dh:(h + 1) * Dh, :],
                            lambda u: qb[(T + u % L) % NQ, it * NBT + u // L],
                            lambda u: wob[(T + u % L) % NW], finish, None)
            nxt = jnp.where(slot == nslot - 1, 0, slot + 1)
            return jnp.where(sub == TS - 1, nxt, slot)

        if only != 1:
            lax.fori_loop(0, L * TS, tail, jnp.int32(T % nslot))
        with scope("w_out"):
            pltpu.make_async_copy(ob, out, sem_o).wait()

    hbm = pl.BlockSpec(memory_space=pl.ANY)

    def fn(A_x, A_k, A_v, A_wq, A_wo, B_x, B_k, B_v, B_wq, B_wo):
        t = lambda a: jnp.swapaxes(a, 2, 3).reshape(B, P, W, Sk)
        w = lambda a: a.reshape(P, W, D)
        DMA = pltpu.SemaphoreType.DMA
        return pl.pallas_call(
            kernel,
            in_specs=[hbm] * 10,
            out_specs=hbm,
            out_shape=jax.ShapeDtypeStruct((B, Sq, 2 * D), bf16),
            scratch_shapes=[
                pltpu.VMEM((2, B, Sq, D), bf16),
                pltpu.VMEM((nslot, B, W, Sk), bf16),
                pltpu.VMEM((nslot, B, W, Sk), bf16),
                pltpu.VMEM((NW, D, W), bf16),
                pltpu.VMEM((NW, W, D), bf16),
                pltpu.VMEM((NQ, B, Sq, W), bf16),
                pltpu.VMEM((2, B, Sq, D), f32),
                pltpu.VMEM((B, Sq, 2 * D), bf16),
                pltpu.VMEM((NS, Sq, Sk), bf16),
                DMA((nslot,)), DMA((nslot,)), DMA((C0 + 2,)), DMA((NW,)), DMA((NW,)), DMA(()),
            ],
            compiler_params=pltpu.CompilerParams(
                vmem_limit_bytes=vmem_mb * 1024 * 1024, flags=flags, disable_bounds_checks=True),
        )(A_x, t(A_k), t(A_v), A_wq, w(A_wo), B_x, t(B_k), t(B_v), B_wq, w(B_wo))
    return fn


@jax.jit
def pallas_concat_heads__gqa_block_cached__mha_block_cached__near_ridge_kernel(
    A_x, A_k_cache, A_v_cache, A_wq, A_wo, B_x, B_k_cache, B_v_cache, B_wq, B_wo
):
    return make(pat='KKFOVV',look=4,olag=2,qlast=2,NS=8,tpat='OKKVV',tlook=2,tolag=5,zpos=4)(
        A_x, A_k_cache, A_v_cache, A_wq, A_wo, B_x, B_k_cache, B_v_cache, B_wq, B_wo)
```

```python
import math

import jax
import jax.numpy as jnp
from jax import lax
import jax.experimental.pallas as pl
import jax.experimental.pallas.tpu as pltpu

_NT = (((1,), (1,)), ((), ()))
_LANES = 128


@jax.jit
def pallas_concat_heads__gqa_block_cached__mha_block_cached__near_ridge_kernel(
    A_x: jax.Array,
    A_k_cache: jax.Array,
    A_v_cache: jax.Array,
    A_wq: jax.Array,
    A_wo: jax.Array,
    B_x: jax.Array,
    B_k_cache: jax.Array,
    B_v_cache: jax.Array,
    B_wq: jax.Array,
    B_wo: jax.Array,
):
    B, Sq, D = A_x.shape
    _, H, Sk, Dh = A_k_cache.shape
    assert (B, H, Dh) == (16, 32, 192) and B_k_cache.shape == A_k_cache.shape
    assert A_wq.shape == (D, H * Dh)
    P = H // 2
    W = 2 * Dh
    LAG = 4
    T = 2 * P - LAG
    NKV = 3
    NQ = LAG + 1
    NW = 8
    NP = 8
    HB = 2
    CB = B // LAG
    TB = CB // 2
    SM = 128
    RC = 16
    q_scale = (Dh ** -0.5) * math.log2(math.e)
    f32, bf16 = jnp.float32, jnp.bfloat16

    def kernel(ax, ak, av, awq, awo, bx, bk, bv, bwq, bwo, out,
               x_buf, kv_buf, wq_buf, wo_buf, q_buf, p_buf, acc, o_buf,
               kv_sem, x_sem, wq_sem, wo_sem, o_sem):
        ks, vs, wqs, wos = (ak, bk), (av, bv), (awq, bwq), (awo, bwo)
        copy = pltpu.make_async_copy

        def start_kv(br, p, slot):
            copy(ks[br].at[:, p], kv_buf.at[slot, 0], kv_sem.at[slot]).start()
            copy(vs[br].at[:, p], kv_buf.at[slot, 1], kv_sem.at[slot]).start()

        def start_kv_tail(c, slot):
            for i in range(CB):
                for j, src in enumerate((bk, bv)):
                    copy(src.at[c * CB + i, pl.ds(P - LAG, LAG)],
                         kv_buf.at[slot, j, pl.ds(i * LAG, LAG)], kv_sem.at[slot]).start()

        def start_wq(br, p, slot):
            col = p * W if isinstance(p, int) else pl.multiple_of(p * W, _LANES)
            copy(wqs[br].at[:, pl.ds(col, W)], wq_buf.at[slot], wq_sem.at[slot]).start()

        def start_wo(br, p, slot):
            copy(wos[br].at[p], wo_buf.at[slot], wo_sem.at[slot]).start()

        def wait_slot(buf, sem, slot):
            copy(buf.at[slot], buf.at[slot], sem.at[slot]).wait()

        def xa_copy(c):
            return copy(ax.at[pl.ds(c * HB, HB)], x_buf.at[0, pl.ds(c * HB, HB)], x_sem.at[c])

        def xb_copy():
            return copy(bx, x_buf.at[1], x_sem.at[B // HB])

        def ring_next(v, n):
            return jnp.where(v == n - 1, 0, v + 1)

        def ring_prev(v, n):
            return jnp.where(v == 0, n - 1, v - 1)

        low_lanes = lax.broadcasted_iota(jnp.int32, (Sq, _LANES), 1) < Dh - _LANES

        def q_proj(x, w):
            return (jnp.dot(x, w, preferred_element_type=f32) * q_scale).astype(bf16)

        def attention_stages(slot, u0, load_wo):
            s, r, o_main, o_rest = {}, {}, {}, {}

            def scores(u, q):
                for h in range(2):
                    s[u, h] = jnp.dot(q[:, h * Dh:(h + 1) * Dh],
                                      kv_buf[slot, 0, u0 + u, h * Dh:(h + 1) * Dh, :],
                                      preferred_element_type=f32)

            def softmax_pv(u):
                for h in range(2):
                    ps = (2 * u + h) % NP
                    s_h = s.pop((u, h))
                    inv = []
                    for r0 in range(0, Sq, RC):
                        s_c = s_h[r0:r0 + RC]
                        m = jnp.max(s_c, axis=-1, keepdims=True)
                        p = jnp.exp2(s_c - m).astype(bf16)
                        inv.append(1.0 / jnp.sum(p.astype(f32), axis=-1, keepdims=True))
                        p_buf[ps, r0:r0 + RC, :] = p
                    r[u, h] = jnp.concatenate(inv, axis=0)
                    p_main, p_rest = p_buf[ps, :SM, :], p_buf[ps, SM:, :]
                    vt = kv_buf[slot, 1, u0 + u, h * Dh:(h + 1) * Dh, :]
                    o_main[u, h] = lax.dot_general(vt, p_main, _NT, preferred_element_type=f32)
                    o_rest[u, h] = lax.dot_general(p_rest, vt, _NT, preferred_element_type=f32)

            def out_proj(u):
                top = jnp.concatenate([o_main.pop((u, 0)), o_main.pop((u, 1))], axis=0)
                rest = jnp.concatenate([o_rest.pop((u, 0)), o_rest.pop((u, 1))], axis=1)
                o = jnp.concatenate([top.T, rest], axis=0)
                r0, r1 = r.pop((u, 0)), r.pop((u, 1))
                o = jnp.concatenate([o[:, :_LANES] * r0,
                                     o[:, _LANES:2 * _LANES] * jnp.where(low_lanes, r0, r1),
                                     o[:, 2 * _LANES:] * r1], axis=1)
                return jnp.dot(o.astype(bf16), load_wo(u), preferred_element_type=f32)

            return scores, softmax_pv, out_proj

        def start_main_inputs(t):
            start_kv(0, t, t)
            start_wo(0, t, t)
            start_wq(0, t + LAG, t + LAG)

        xa_copy(0).start()
        start_wq(0, 0, 0)

        def zero_acc(b, carry):
            acc[0, b] = jnp.zeros((Sq, D), f32)
            acc[1, b] = jnp.zeros((Sq, D), f32)

            @pl.when(b == B // 4)
            def _():
                start_wq(0, 1, 1)

            return carry

        lax.fori_loop(0, B, zero_acc, 0)
        xa_copy(0).wait()

        def head_first_batches(j, carry):
            wait_slot(wq_buf, wq_sem, j)

            @pl.when(j + 2 < LAG)
            def _():
                start_wq(0, j + 2, j + 2)

            @pl.when(j + 2 == LAG)
            def _():
                xa_copy(1).start()
                xa_copy(2).start()

            @pl.when(j + 1 == LAG)
            def _():
                for c in range(3, B // HB):
                    xa_copy(c).start()

            for b in range(HB):
                q_buf[j, b] = q_proj(x_buf[0, b], wq_buf[j])
            return carry

        lax.fori_loop(0, LAG, head_first_batches, 0)

        def head_other_batches(c, carry):
            xa_copy(c).wait()

            @pl.when(c == 2)
            def _():
                start_main_inputs(0)

            for i in range(HB):
                b = c * HB + i
                for j in range(LAG):
                    q_buf[j, b] = q_proj(x_buf[0, b], wq_buf[j])
            return carry

        lax.fori_loop(1, B // HB, head_other_batches, 0)
        for t in range(1, NKV - 1):
            start_main_inputs(t)
        xb_copy().start()

        def main(t, carry):
            slot, q_rd, q_wr = carry
            tq = t + LAG

            @pl.when(tq == P)
            def _():
                xb_copy().wait()

            wait_slot(wo_buf, wo_sem, t & (NW - 1))
            wait_slot(wq_buf, wq_sem, tq & (NW - 1))
            wait_slot(kv_buf, kv_sem, slot)

            def prefetch():
                tn = t + (NKV - 1)
                free = ring_prev(slot, NKV)
                for br in range(2):
                    @pl.when(jnp.logical_and(tn >= br * P, tn < min((br + 1) * P, T)))
                    def _():
                        start_kv(br, tn - br * P, free)
                        start_wo(br, tn - br * P, tn & (NW - 1))

                    @pl.when(jnp.logical_and(tn + LAG >= br * P, tn + LAG < (br + 1) * P))
                    def _():
                        start_wq(br, tn + LAG - br * P, (tn + LAG) & (NW - 1))

                @pl.when(tn >= T)
                def _():
                    start_kv_tail(tn - T, free)

                @pl.when(tn == T)
                def _():
                    for j in range(LAG):
                        start_wo(1, P - LAG + j, (T + j) % NW)

            br_att, br_q = lax.div(t, P), lax.div(tq, P)
            scores, softmax_pv, out_proj = attention_stages(
                slot, 0, lambda u: wo_buf[t & (NW - 1)])

            def accumulate(u):
                acc[br_att, u] += out_proj(u)

            def project_ahead(u):
                q_buf[q_wr, u] = q_proj(x_buf[br_q, u], wq_buf[tq & (NW - 1)])

            scores(0, q_buf[q_rd, 0])
            scores(1, q_buf[q_rd, 1])
            q_next = q_buf[q_rd, 2]
            for u in range(B):
                if u + 2 < B:
                    scores(u + 2, q_next)
                    if u + 3 < B:
                        q_next = q_buf[q_rd, u + 3]
                    if u == 0:
                        prefetch()
                    project_ahead(u)
                if u >= 2:
                    accumulate(u - 2)
                softmax_pv(u)
            for u in (B - 2, B - 1):
                accumulate(u)
            for u in (B - 2, B - 1):
                project_ahead(u)
            return ring_next(slot, NKV), ring_next(q_rd, NQ), ring_next(q_wr, NQ)

        lax.fori_loop(0, T, main, (jnp.int32(0), jnp.int32(0), jnp.int32(LAG)))

        for j in range(LAG):
            wait_slot(wo_buf, wo_sem, (T + j) % NW)

        def tail(it, slot):
            c, half = it >> 1, it & 1
            U = TB * LAG

            @pl.when(half == 0)
            def _():
                wait_slot(kv_buf, kv_sem, slot)

            scores, softmax_pv, out_proj = attention_stages(
                slot, half * U, lambda u: wo_buf[(T + u % LAG) % NW])

            def load_q(u):
                return q_buf[(T + u % LAG) % NQ, it * TB + u // LAG]

            def accumulate(u):
                y = out_proj(u)
                b = it * TB + u // LAG
                if u == 0:
                    @pl.when(jnp.logical_and(half == 0, c + (NKV - 1) < LAG))
                    def _():
                        start_kv_tail(c + (NKV - 1), ring_prev(slot, NKV))
                if u % LAG < LAG - 1:
                    acc[1, b] += y
                else:
                    o_buf[b, :, :D] = acc[0, b].astype(bf16)
                    o_buf[b, :, D:] = (acc[1, b] + y).astype(bf16)
                    copy(o_buf.at[b], out.at[b], o_sem).start()

            scores(0, load_q(0))
            for u in range(U):
                if u >= 4:
                    accumulate(u - 4)
                if u + 1 < U:
                    scores(u + 1, load_q(u + 1))
                softmax_pv(u)
            for u in range(U - 4, U):
                accumulate(u)
            return jnp.where(half == 1, ring_next(slot, NKV), slot)

        lax.fori_loop(0, B // TB, tail, jnp.int32(T % NKV))
        copy(o_buf, out, o_sem).wait()

    def kv_arg(a):
        return jnp.swapaxes(a, 2, 3).reshape(B, P, W, Sk)

    hbm = pl.BlockSpec(memory_space=pl.ANY)
    dma = pltpu.SemaphoreType.DMA
    return pl.pallas_call(
        kernel,
        in_specs=[hbm] * 10,
        out_specs=hbm,
        out_shape=jax.ShapeDtypeStruct((B, Sq, 2 * D), bf16),
        scratch_shapes=[
            pltpu.VMEM((2, B, Sq, D), bf16),
            pltpu.VMEM((NKV, 2, B, W, Sk), bf16),
            pltpu.VMEM((NW, D, W), bf16),
            pltpu.VMEM((NW, W, D), bf16),
            pltpu.VMEM((NQ, B, Sq, W), bf16),
            pltpu.VMEM((NP, Sq, Sk), bf16),
            pltpu.VMEM((2, B, Sq, D), f32),
            pltpu.VMEM((B, Sq, 2 * D), bf16),
            dma((NKV,)), dma((B // HB + 1,)), dma((NW,)), dma((NW,)), dma(()),
        ],
        compiler_params=pltpu.CompilerParams(
            vmem_limit_bytes=120 * 1024 * 1024, disable_bounds_checks=True),
    )(A_x, kv_arg(A_k_cache), kv_arg(A_v_cache), A_wq, A_wo.reshape(P, W, D),
      B_x, kv_arg(B_k_cache), kv_arg(B_v_cache), B_wq, B_wo.reshape(P, W, D))
```

```python
import math

import jax
import jax.numpy as jnp
from jax import lax
import jax.experimental.pallas as pl
import jax.experimental.pallas.tpu as pltpu

_NT = (((1,), (1,)), ((), ()))
_LANES = 128


@jax.jit
def pallas_concat_heads__gqa_block_cached__mha_block_cached__near_ridge_kernel(
    A_x: jax.Array,
    A_k_cache: jax.Array,
    A_v_cache: jax.Array,
    A_wq: jax.Array,
    A_wo: jax.Array,
    B_x: jax.Array,
    B_k_cache: jax.Array,
    B_v_cache: jax.Array,
    B_wq: jax.Array,
    B_wo: jax.Array,
):
    B, Sq, D = A_x.shape
    _, H, Sk, Dh = A_k_cache.shape
    assert (B, H, Dh) == (16, 32, 192) and B_k_cache.shape == A_k_cache.shape
    assert A_wq.shape == (D, H * Dh)
    P = H // 2
    W = 2 * Dh
    LAG = 4
    T = 2 * P - LAG
    NKV = 3
    NQ = LAG + 1
    NW = 8
    NP = 8
    HB = 4
    CB = B // LAG
    TB = CB // 2
    SM = 128
    RC = 16
    q_scale = (Dh ** -0.5) * math.log2(math.e)
    f32, bf16 = jnp.float32, jnp.bfloat16

    def kernel(ax, ak, av, awq, awo, bx, bk, bv, bwq, bwo, out,
               x_buf, kv_buf, wq_buf, wo_buf, q_buf, p_buf, acc, o_buf,
               kv_sem, x_sem, wq_sem, wo_sem, o_sem):
        ks, vs, wqs, wos = (ak, bk), (av, bv), (awq, bwq), (awo, bwo)
        copy = pltpu.make_async_copy

        def start_kv(br, p, slot):
            copy(ks[br].at[:, p], kv_buf.at[slot, 0], kv_sem.at[slot]).start()
            copy(vs[br].at[:, p], kv_buf.at[slot, 1], kv_sem.at[slot]).start()

        def start_kv_tail(c, slot):
            for i in range(CB):
                for j, src in enumerate((bk, bv)):
                    copy(src.at[c * CB + i, pl.ds(P - LAG, LAG)],
                         kv_buf.at[slot, j, pl.ds(i * LAG, LAG)], kv_sem.at[slot]).start()

        def start_wq(br, p, slot):
            col = p * W if isinstance(p, int) else pl.multiple_of(p * W, _LANES)
            copy(wqs[br].at[:, pl.ds(col, W)], wq_buf.at[slot], wq_sem.at[slot]).start()

        def start_wo(br, p, slot):
            copy(wos[br].at[p], wo_buf.at[slot], wo_sem.at[slot]).start()

        def wait_slot(buf, sem, slot):
            copy(buf.at[slot], buf.at[slot], sem.at[slot]).wait()

        def xa_copy(c):
            return copy(ax.at[pl.ds(c * HB, HB)], x_buf.at[0, pl.ds(c * HB, HB)], x_sem.at[c])

        def xb_copy():
            return copy(bx, x_buf.at[1], x_sem.at[B // HB])

        def ring_next(v, n):
            return jnp.where(v == n - 1, 0, v + 1)

        def ring_prev(v, n):
            return jnp.where(v == 0, n - 1, v - 1)

        low_lanes = lax.broadcasted_iota(jnp.int32, (Sq, _LANES), 1) < Dh - _LANES

        def q_proj(x, w):
            return (jnp.dot(x, w, preferred_element_type=f32) * q_scale).astype(bf16)

        def attention_stages(slot, u0, load_wo):
            s, r, o_main, o_rest = {}, {}, {}, {}

            def scores(u, q):
                for h in range(2):
                    s[u, h] = jnp.dot(q[:, h * Dh:(h + 1) * Dh],
                                      kv_buf[slot, 0, u0 + u, h * Dh:(h + 1) * Dh, :],
                                      preferred_element_type=f32)

            def softmax_pv(u):
                for h in range(2):
                    ps = (2 * u + h) % NP
                    s_h = s.pop((u, h))
                    inv = []
                    for r0 in range(0, Sq, RC):
                        s_c = s_h[r0:r0 + RC]
                        m = jnp.max(s_c, axis=-1, keepdims=True)
                        p = jnp.exp2(s_c - m).astype(bf16)
                        inv.append(1.0 / jnp.sum(p.astype(f32), axis=-1, keepdims=True))
                        p_buf[ps, r0:r0 + RC, :] = p
                    r[u, h] = jnp.concatenate(inv, axis=0)
                    p_main, p_rest = p_buf[ps, :SM, :], p_buf[ps, SM:, :]
                    vt = kv_buf[slot, 1, u0 + u, h * Dh:(h + 1) * Dh, :]
                    o_main[u, h] = lax.dot_general(vt, p_main, _NT, preferred_element_type=f32)
                    o_rest[u, h] = lax.dot_general(p_rest, vt, _NT, preferred_element_type=f32)

            def out_proj(u):
                top = jnp.concatenate([o_main.pop((u, 0)), o_main.pop((u, 1))], axis=0)
                rest = jnp.concatenate([o_rest.pop((u, 0)), o_rest.pop((u, 1))], axis=1)
                o = jnp.concatenate([top.T, rest], axis=0)
                r0, r1 = r.pop((u, 0)), r.pop((u, 1))
                o = jnp.concatenate([o[:, :_LANES] * r0,
                                     o[:, _LANES:2 * _LANES] * jnp.where(low_lanes, r0, r1),
                                     o[:, 2 * _LANES:] * r1], axis=1)
                return jnp.dot(o.astype(bf16), load_wo(u), preferred_element_type=f32)

            return scores, softmax_pv, out_proj

        def start_main_inputs(t):
            start_kv(0, t, t)
            start_wo(0, t, t)
            start_wq(0, t + LAG, t + LAG)

        xa_copy(0).start()
        start_wq(0, 0, 0)

        def zero_acc(b, carry):
            acc[0, b] = jnp.zeros((Sq, D), f32)
            acc[1, b] = jnp.zeros((Sq, D), f32)

            @pl.when(b == B // 4)
            def _():
                start_wq(0, 1, 1)

            return carry

        lax.fori_loop(0, B, zero_acc, 0)
        xa_copy(0).wait()

        def head_first_batches(j, carry):
            wait_slot(wq_buf, wq_sem, j)

            @pl.when(j + 2 < LAG)
            def _():
                start_wq(0, j + 2, j + 2)

            @pl.when(j + 2 == LAG)
            def _():
                xa_copy(1).start()
                xa_copy(2).start()

            @pl.when(j + 1 == LAG)
            def _():
                for c in range(3, B // HB):
                    xa_copy(c).start()

            for b in range(HB):
                q_buf[j, b] = q_proj(x_buf[0, b], wq_buf[j])
            return carry

        lax.fori_loop(0, LAG, head_first_batches, 0)

        def head_other_batches(c, carry):
            xa_copy(c).wait()

            @pl.when(c == 1)
            def _():
                start_main_inputs(0)

            for i in range(HB):
                b = c * HB + i
                for j in range(LAG):
                    q_buf[j, b] = q_proj(x_buf[0, b], wq_buf[j])
            return carry

        lax.fori_loop(1, B // HB, head_other_batches, 0)
        for t in range(1, NKV - 1):
            start_main_inputs(t)
        xb_copy().start()

        def main(t, carry):
            slot, q_rd, q_wr = carry
            tq = t + LAG

            @pl.when(tq == P)
            def _():
                xb_copy().wait()

            wait_slot(wo_buf, wo_sem, t & (NW - 1))
            wait_slot(wq_buf, wq_sem, tq & (NW - 1))
            wait_slot(kv_buf, kv_sem, slot)

            def prefetch():
                tn = t + (NKV - 1)
                free = ring_prev(slot, NKV)
                for br in range(2):
                    @pl.when(jnp.logical_and(tn >= br * P, tn < min((br + 1) * P, T)))
                    def _():
                        start_kv(br, tn - br * P, free)
                        start_wo(br, tn - br * P, tn & (NW - 1))

                    @pl.when(jnp.logical_and(tn + LAG >= br * P, tn + LAG < (br + 1) * P))
                    def _():
                        start_wq(br, tn + LAG - br * P, (tn + LAG) & (NW - 1))

                @pl.when(tn >= T)
                def _():
                    start_kv_tail(tn - T, free)

                @pl.when(tn == T)
                def _():
                    for j in range(LAG):
                        start_wo(1, P - LAG + j, (T + j) % NW)

            br_att, br_q = lax.div(t, P), lax.div(tq, P)
            scores, softmax_pv, out_proj = attention_stages(
                slot, 0, lambda u: wo_buf[t & (NW - 1)])

            def accumulate(u):
                acc[br_att, u] += out_proj(u)

            def project_ahead(u):
                q_buf[q_wr, u] = q_proj(x_buf[br_q, u], wq_buf[tq & (NW - 1)])

            scores(0, q_buf[q_rd, 0])
            scores(1, q_buf[q_rd, 1])
            q_next = q_buf[q_rd, 2]
            for u in range(B):
                if u + 2 < B:
                    scores(u + 2, q_next)
                    if u + 3 < B:
                        q_next = q_buf[q_rd, u + 3]
                    if u == 0:
                        prefetch()
                    project_ahead(u)
                if u >= 2:
                    accumulate(u - 2)
                softmax_pv(u)
            for u in (B - 2, B - 1):
                accumulate(u)
            for u in (B - 2, B - 1):
                project_ahead(u)
            return ring_next(slot, NKV), ring_next(q_rd, NQ), ring_next(q_wr, NQ)

        lax.fori_loop(0, T, main, (jnp.int32(0), jnp.int32(0), jnp.int32(LAG)))

        for j in range(LAG):
            wait_slot(wo_buf, wo_sem, (T + j) % NW)

        def write_out(b, br, y):
            cols = pl.ds(br * D, D)
            o_buf[b, :, cols] = y.astype(bf16)
            copy(o_buf.at[b, :, cols], out.at[b, :, cols], o_sem).start()

        def tail(it, slot):
            c, half = it >> 1, it & 1
            U = TB * LAG

            @pl.when(half == 0)
            def _():
                wait_slot(kv_buf, kv_sem, slot)

            scores, softmax_pv, out_proj = attention_stages(
                slot, half * U, lambda u: wo_buf[(T + u % LAG) % NW])

            def load_q(u):
                return q_buf[(T + u % LAG) % NQ, it * TB + u // LAG]

            def accumulate(u):
                y = out_proj(u)
                b = it * TB + u // LAG
                if u == 0:
                    @pl.when(jnp.logical_and(half == 0, c + (NKV - 1) < LAG))
                    def _():
                        start_kv_tail(c + (NKV - 1), ring_prev(slot, NKV))
                if u % LAG == 0:
                    write_out(b, 0, acc[0, b])
                if u % LAG < LAG - 1:
                    acc[1, b] += y
                else:
                    write_out(b, 1, acc[1, b] + y)

            scores(0, load_q(0))
            for u in range(U):
                if u >= 4:
                    accumulate(u - 4)
                if u + 1 < U:
                    scores(u + 1, load_q(u + 1))
                softmax_pv(u)
            for u in range(U - 4, U):
                accumulate(u)
            return jnp.where(half == 1, ring_next(slot, NKV), slot)

        lax.fori_loop(0, B // TB, tail, jnp.int32(T % NKV))
        copy(o_buf, out, o_sem).wait()

    def kv_arg(a):
        return jnp.swapaxes(a, 2, 3).reshape(B, P, W, Sk)

    hbm = pl.BlockSpec(memory_space=pl.ANY)
    dma = pltpu.SemaphoreType.DMA
    return pl.pallas_call(
        kernel,
        in_specs=[hbm] * 10,
        out_specs=hbm,
        out_shape=jax.ShapeDtypeStruct((B, Sq, 2 * D), bf16),
        scratch_shapes=[
            pltpu.VMEM((2, B, Sq, D), bf16),
            pltpu.VMEM((NKV, 2, B, W, Sk), bf16),
            pltpu.VMEM((NW, D, W), bf16),
            pltpu.VMEM((NW, W, D), bf16),
            pltpu.VMEM((NQ, B, Sq, W), bf16),
            pltpu.VMEM((NP, Sq, Sk), bf16),
            pltpu.VMEM((2, B, Sq, D), f32),
            pltpu.VMEM((B, Sq, 2 * D), bf16),
            dma((NKV,)), dma((B // HB + 1,)), dma((NW,)), dma((NW,)), dma(()),
        ],
        compiler_params=pltpu.CompilerParams(
            vmem_limit_bytes=100 * 1024 * 1024, disable_bounds_checks=True),
    )(A_x, kv_arg(A_k_cache), kv_arg(A_v_cache), A_wq, A_wo.reshape(P, W, D),
      B_x, kv_arg(B_k_cache), kv_arg(B_v_cache), B_wq, B_wo.reshape(P, W, D))
```
